```python
import jax
import jax.numpy as jnp

def _softmax(x, axis=-1):
    return jax.nn.softmax(x, axis=axis)
def _gelu(x):
    return jax.nn.gelu(x, approximate=True)
def _silu(x):
    return jax.nn.silu(x)
def _sigmoid(x):
    return jax.nn.sigmoid(x)
def _layernorm(x, axis=-1, eps=1e-5):
    m = jnp.mean(x, axis=axis, keepdims=True)
    v = jnp.var(x, axis=axis, keepdims=True)
    return (x - m) / jnp.sqrt(v + eps)
def _scatter_add(tgt, idx, src, axis=0):
    return tgt.at[idx].add(src)
def _segment_sum(src, seg, n):
    return jax.ops.segment_sum(src, seg, n)
class _Rng:
    def __init__(self, key):
        self._k = key
    def _next(self):
        self._k, sub = jax.random.split(self._k)
        return sub
    def normal(self, shape):
        return jax.random.normal(self._next(), shape, dtype=jnp.bfloat16)
    def randint(self, lo, hi, shape):
        return jax.random.randint(self._next(), shape, lo, hi, dtype=jnp.int32)
    def uniform(self, shape, lo=0.0, hi=1.0):
        return jax.random.uniform(self._next(), shape, jnp.bfloat16, lo, hi)
    def permutation(self, n):
        return jax.random.permutation(self._next(), n)


kernel_name = 'standalone__detection_seg_fpn_lateral__vision'

def setup_inputs():
    _rng = _Rng(jax.random.key(int.from_bytes(__import__("os").urandom(4), "little")))
    _w = (lambda a: (lambda t: t.astype(jnp.bfloat16) if jnp.issubdtype(t.dtype, jnp.floating) else t)(jnp.asarray(a)))
    H = W = (384 // 2) * 2
    C = 384
    k = 1
    return {
        "c_fine": _w((lambda *s: _rng.normal(s) * 0.05)(1, H, W, C)),
        "p_coarse": _w((lambda *s: _rng.normal(s) * 0.05)(1, H // 2, W // 2, C)),
        "w_lat": _w((lambda *s: _rng.normal(s) * 0.05)(C, C)),
        "w_out": _w((lambda *s: _rng.normal(s) * 0.05)(k, k, C, C)),
    }

def reference(c_fine, p_coarse, w_lat, w_out):
    B, H, W, C = c_fine.shape
    k = 1
    lat = jnp.einsum("bhwc,cd->bhwd", c_fine, w_lat)
    up = jnp.repeat(jnp.repeat(p_coarse, 2, axis=1), 2, axis=2)
    m = lat + up
    pad = k // 2
    mp = jnp.pad(m, ((0, 0), (pad, pad), (pad, pad), (0, 0)))
    o = None
    for di in range(k):
        for dj in range(k):
            t = jnp.einsum("bhwc,cd->bhwd", mp[:, di:di + H, dj:dj + W, :], w_out[di, dj])
            o = t if o is None else o + t
    return o
```

```python
import functools

import jax
import jax.numpy as jnp
import jax.experimental.pallas as pl
import jax.experimental.pallas.tpu as pltpu


def _kernel(c_ref, p_ref, wl_ref, wo_ref, o_ref, wf_ref, up_ref, *, th):
    W = c_ref.shape[1]
    C = c_ref.shape[2]
    nt = C // 128

    @pl.when(pl.program_id(0) == 0)
    def _():
        wf_ref[...] = jnp.dot(
            wl_ref[...], wo_ref[...], preferred_element_type=jnp.float32
        ).astype(jnp.bfloat16)

    def body(i, carry):
        q = jnp.dot(p_ref[i], wo_ref[...], preferred_element_type=jnp.float32)
        for n in range(nt):
            qn = q[:, n * 128:(n + 1) * 128]
            up_ref[n, pl.ds(0, W // 2, stride=2), :] = qn
            up_ref[n, pl.ds(1, W // 2, stride=2), :] = qn
        for r in range(2):
            acc = jnp.dot(c_ref[2 * i + r], wf_ref[...], preferred_element_type=jnp.float32)
            up = jnp.concatenate([up_ref[n] for n in range(nt)], axis=1)
            o_ref[2 * i + r] = (acc + up).astype(o_ref.dtype)
        return carry

    jax.lax.fori_loop(0, th // 2, body, 0)


@jax.jit
def pallas_standalone__detection_seg_fpn_lateral__vision_kernel(
    c_fine: jax.Array,
    p_coarse: jax.Array,
    w_lat: jax.Array,
    w_out: jax.Array,
):
    B, H, W, C = c_fine.shape
    th = 8
    c3 = c_fine.reshape(B * H, W, C)
    p3 = p_coarse.reshape(B * H // 2, W // 2, C)
    wo = w_out.reshape(C, C)
    out = pl.pallas_call(
        functools.partial(_kernel, th=th),
        grid=(B * H // th,),
        in_specs=[
            pl.BlockSpec((th, W, C), lambda i: (i, 0, 0)),
            pl.BlockSpec((th // 2, W // 2, C), lambda i: (i, 0, 0)),
            pl.BlockSpec((C, C), lambda i: (0, 0)),
            pl.BlockSpec((C, C), lambda i: (0, 0)),
        ],
        out_specs=pl.BlockSpec((th, W, C), lambda i: (i, 0, 0)),
        out_shape=jax.ShapeDtypeStruct((B * H, W, C), c_fine.dtype),
        scratch_shapes=[
            pltpu.VMEM((C, C), jnp.bfloat16),
            pltpu.VMEM((C // 128, W, 128), jnp.float32),
        ],
        compiler_params=pltpu.CompilerParams(
            dimension_semantics=("arbitrary",),
            vmem_limit_bytes=64 * 1024 * 1024,
        ),
    )(c3, p3, w_lat, wo)
    return out.reshape(B, H, W, C)
```

```python
import functools

import jax
import jax.numpy as jnp
import jax.experimental.pallas as pl
import jax.experimental.pallas.tpu as pltpu

U = 4
PRING = 24
WG = 6
BW = 48
I0 = 112
G0 = 4
GSTEP = 3
SCOPES = False


class _NoScope:
    def __enter__(self):
        return self

    def __exit__(self, *a):
        return False


def _scope(name):
    return jax.named_scope(name) if SCOPES else _NoScope()


def _kernel(c_hbm, p_hbm, wl_hbm, wo_hbm, o_hbm,
            cbuf, pbuf, wl_v, wo_v, wf_v, up_ref, csem, psem, wsem, ksem,
            *, u, pring, wg, bw, i0, g0, gstep):
    npairs, w2, C = c_hbm.shape
    W = w2 // 2
    nt = C // 128
    nu = npairs // u
    ns = w2 // bw
    ng = npairs // wg
    n_in_loop = g0 + (npairs - 1 - i0) // gstep
    assert n_in_loop <= ng
    for t in range(i0, npairs):
        issued = g0 + (t - i0) // gstep
        assert issued * wg <= t, (t, issued)
    assert nu - pring <= i0 // u

    def rd_c(un):
        return pltpu.make_async_copy(
            c_hbm.at[pl.ds(un * u, u)], cbuf.at[pl.ds(un * u, u)], csem.at[un % pring])

    def rd_p(un):
        s = un % pring
        return pltpu.make_async_copy(
            p_hbm.at[pl.ds(un * u, u)], pbuf.at[pl.ds(s * u, u)], psem.at[s])

    def start_unit(un):
        rd_c(un).start()
        rd_p(un).start()

    def start_group(g):
        def issue(j, carry):
            off = pl.multiple_of(j * bw, bw)
            pltpu.make_async_copy(
                cbuf.at[pl.ds(g * wg, wg), pl.ds(off, bw)],
                o_hbm.at[pl.ds(g * wg, wg), pl.ds(off, bw)], wsem).start()
            return carry
        jax.lax.fori_loop(0, ns, issue, 0)

    def start_groups(lo, hi):
        def issue(g, carry):
            start_group(g)
            return carry
        jax.lax.fori_loop(lo, hi, issue, 0)

    wl_cp = pltpu.make_async_copy(wl_hbm, wl_v, ksem.at[0])
    wo_cp = pltpu.make_async_copy(wo_hbm, wo_v, ksem.at[1])
    wl_cp.start()
    wo_cp.start()

    def pro(un, carry):
        start_unit(un)
        return carry
    jax.lax.fori_loop(0, pring, pro, 0)

    with _scope("fold"):
        wl_cp.wait()
        wo_cp.wait()
        wf_v[...] = jnp.dot(wl_v[...], wo_v[...],
                            preferred_element_type=jnp.float32).astype(jnp.bfloat16)

    def pair(i, carry):
        un = i // u

        @pl.when(i % u == 0)
        def _():
            @pl.when(jnp.logical_and(un >= 1, un + pring - 1 < nu))
            def _():
                start_unit(un + pring - 1)

            with _scope("waitU"):
                @pl.when(un < nu - 1)
                def _():
                    rd_c(un).wait()
                rd_p(un).wait()

        @pl.when(i == i0)
        def _():
            with _scope("waitR"):
                rd_c(nu - 1).wait()
            with _scope("startW"):
                start_groups(0, g0)

        @pl.when(jnp.logical_and(i > i0, (i - i0) % gstep == 0))
        def _():
            with _scope("startG"):
                start_group(g0 - 1 + (i - i0) // gstep)

        q = jnp.dot(pbuf[(un % pring) * u + i % u], wo_v[...], preferred_element_type=jnp.float32)
        for n in range(nt):
            qn = q[:, n * 128:(n + 1) * 128]
            up_ref[n, pl.ds(0, W // 2, stride=2), :] = qn
            up_ref[n, pl.ds(1, W // 2, stride=2), :] = qn
        for h in range(2):
            acc = jnp.dot(cbuf[i, pl.ds(h * W, W), :], wf_v[...],
                          preferred_element_type=jnp.float32)
            up = jnp.concatenate([up_ref[n] for n in range(nt)], axis=1)
            cbuf[i, pl.ds(h * W, W), :] = (acc + up).astype(cbuf.dtype)
        return carry

    with _scope("compute"):
        jax.lax.fori_loop(0, npairs, pair, 0)
    with _scope("tail"):
        start_groups(n_in_loop, ng)
        pltpu.make_async_copy(cbuf, o_hbm, wsem).wait()


@jax.jit
def pallas_standalone__detection_seg_fpn_lateral__vision_kernel(
    c_fine: jax.Array,
    p_coarse: jax.Array,
    w_lat: jax.Array,
    w_out: jax.Array,
):
    B, H, W, C = c_fine.shape
    npairs = B * H // 2
    c3 = c_fine.reshape(npairs, 2 * W, C)
    p3 = p_coarse.reshape(npairs, W // 2, C)
    wo = w_out.reshape(C, C)
    any_spec = pl.BlockSpec(memory_space=pl.ANY)
    out = pl.pallas_call(
        functools.partial(_kernel, u=U, pring=PRING, wg=WG, bw=BW, i0=I0, g0=G0, gstep=GSTEP),
        in_specs=[any_spec] * 4,
        out_specs=any_spec,
        out_shape=jax.ShapeDtypeStruct((npairs, 2 * W, C), c_fine.dtype),
        scratch_shapes=[
            pltpu.VMEM((npairs, 2 * W, C), jnp.bfloat16),
            pltpu.VMEM((PRING * U, W // 2, C), jnp.bfloat16),
            pltpu.VMEM((C, C), jnp.bfloat16),
            pltpu.VMEM((C, C), jnp.bfloat16),
            pltpu.VMEM((C, C), jnp.bfloat16),
            pltpu.VMEM((C // 128, W, 128), jnp.float32),
            pltpu.SemaphoreType.DMA((PRING,)),
            pltpu.SemaphoreType.DMA((PRING,)),
            pltpu.SemaphoreType.DMA(()),
            pltpu.SemaphoreType.DMA((2,)),
        ],
        compiler_params=pltpu.CompilerParams(vmem_limit_bytes=127 * 1024 * 1024),
    )(c3, p3, w_lat, wo)
    return out.reshape(B, H, W, C)
```

```python
import functools

import jax
import jax.numpy as jnp
import jax.experimental.pallas as pl
import jax.experimental.pallas.tpu as pltpu

CFG = dict(
    ur=2,
    u=4,
    cq=4,
    pring=96,
    pr=32,
    ni=10,
    sa=57,
    wg=6,
    bw=48,
    s0=32,
    spi=11,
    mc=96,
    qc=96,
    lead=1,
)
SCOPES = False


class _NoScope:
    def __enter__(self):
        return self

    def __exit__(self, *a):
        return False


def _scope(name):
    return jax.named_scope(name) if SCOPES else _NoScope()


def _kernel(c_hbm, p_hbm, wl_hbm, wo_hbm, o_hbm,
            cbuf, pbuf, wl_v, wo_v, wf_v, up_ref, csem, psem, wsem, ksem,
            *, ur, u, cq, pring, pr, ni, sa, wg, bw, s0, spi, mc, qc, lead):
    npairs, w2, C = c_hbm.shape
    W = w2 // 2
    WP = W // 2
    nt = C // 128
    nit = npairs // ur
    nu = npairs // u
    ipu = u // ur
    ns = w2 // bw
    nstrips = (npairs // wg) * ns
    ptot = npairs * WP
    rs = pring * WP
    fpi = ni * pr * ur
    f0 = ptot - fpi * sa
    assert u % ur == 0 and npairs % u == 0
    assert f0 >= ur * WP and f0 % pr == 0 and rs % pr == 0 and f0 <= rs
    assert fpi >= ur * WP
    for it in range(sa):
        assert f0 + fpi * (it + 1) - rs <= ur * it * WP
    assert cq + sa - 1 >= nu
    n_in_loop = s0 + spi * (nit - sa)
    assert n_in_loop <= nstrips
    for it in range(sa, nit):
        hi = s0 + spi * (it - sa + 1)
        assert -(-hi // ns) * wg <= it * ur, it
    anchor = rs

    def c_copy(lo, n, s):
        return pltpu.make_async_copy(
            c_hbm.at[pl.ds(lo, n)], cbuf.at[pl.ds(lo, n)], csem.at[s])

    def rd_c(un):
        return c_copy(un * u, u, un)

    first_a = lambda: c_copy(0, ur, 0)
    first_b = lambda: c_copy(ur, u - ur, nu)
    last_a = lambda: c_copy(npairs - u, u - lead, nu - 1)
    last_b = lambda: c_copy(npairs - lead, lead, nu + 1)

    def p_copy(src, dst, n, s):
        return pltpu.make_async_copy(
            p_hbm.at[pl.ds(src, n)], pbuf.at[pl.ds(dst, n)], psem.at[s])

    def strip(t):
        g = t // ns
        off = pl.multiple_of((t % ns) * bw, bw)
        return pltpu.make_async_copy(
            cbuf.at[pl.ds(g * wg, wg), pl.ds(off, bw)],
            o_hbm.at[pl.ds(g * wg, wg), pl.ds(off, bw)], wsem)

    def start_strips(lo, hi):
        def issue(t, carry):
            strip(t).start()
            return carry
        jax.lax.fori_loop(lo, hi, issue, 0)

    wl_cp = pltpu.make_async_copy(wl_hbm, wl_v, ksem.at[0])
    wo_cp = pltpu.make_async_copy(wo_hbm, wo_v, ksem.at[1])
    wl_cp.start()
    wo_cp.start()
    p_first = p_copy(0, 0, f0, sa)
    p_first.start()

    def pro_c(un, carry):
        @pl.when(un == 0)
        def _():
            first_a().start(priority=1)
            if u > ur:
                first_b().start(priority=1)

        @pl.when(un > 0)
        def _():
            rd_c(un).start(priority=1)
        return carry
    jax.lax.fori_loop(0, cq, pro_c, 0)

    with _scope("fold"):
        wl_cp.wait()
        wo_cp.wait()
        wf_v[...] = jnp.dot(
            wl_v[...], wo_v[...],
            preferred_element_type=jnp.float32).astype(jnp.bfloat16)
        p_first.wait()
        first_a().wait()

    def c_waits(it):
        un = it // ipu
        if u > ur:
            @pl.when(it == 1)
            def _():
                first_b().wait()

        @pl.when(jnp.logical_and(it % ipu == 0, jnp.logical_and(un > 0, un < nu - 1)))
        def _():
            rd_c(un).wait()

    def p_wait(it, jw):
        need = f0 + fpi * jw < ur * WP * (it + 1)

        @pl.when(need)
        def _():
            p_copy(0, 0, fpi, jw).wait()
        return jw + need.astype(jnp.int32)

    def compute(it, pins):
        pins = iter(pins)

        def pin(tile):
            f = next(pins)
            if f is not None:
                if tile is not None:
                    pbuf[pl.ds(anchor, 16), pl.ds(0, 128)] = tile
                f()

        prows = []
        for k in range(ur):
            i = it * ur + k
            prow = pl.multiple_of((i % pring) * WP, WP)
            prows.append(pbuf[pl.ds(prow, WP), :])
        pin(None)
        for k in range(ur):
            i = it * ur + k
            for ch in range(WP // qc):
                q = jnp.dot(prows[k][ch * qc:(ch + 1) * qc], wo_v[...],
                            preferred_element_type=jnp.float32)
                for n in range(nt):
                    qn = q[:, n * 128:(n + 1) * 128]
                    up_ref[k, n, pl.ds(2 * ch * qc, qc, stride=2), :] = qn
                    up_ref[k, n, pl.ds(2 * ch * qc + 1, qc, stride=2), :] = qn
                pin(q[0:16, 0:128].astype(jnp.bfloat16))
            for ch in range(w2 // mc):
                acc = jnp.dot(cbuf[i, pl.ds(ch * mc, mc), :], wf_v[...],
                              preferred_element_type=jnp.float32)
                uo = (ch * mc) % W
                up = jnp.concatenate([up_ref[k, n, pl.ds(uo, mc), :] for n in range(nt)], axis=1)
                res = (acc + up).astype(cbuf.dtype)
                cbuf[i, pl.ds(ch * mc, mc), :] = res
                if not (k == ur - 1 and ch == w2 // mc - 1):
                    pin(res[0:16, 0:128])

    nslots = ur * (WP // qc + w2 // mc)

    def step_a(it, jw):
        un = it + cq

        @pl.when(un < nu - 1)
        def _():
            rd_c(un).start(priority=1)

        @pl.when(un == nu - 1)
        def _():
            last_a().start(priority=1)
            last_b().start(priority=1)

        c_waits(it)
        jw = p_wait(it, jw)
        base = f0 + fpi * it

        def mk(lo, hi):
            def f():
                for k in range(lo, hi):
                    src = pl.multiple_of(base + k * pr, pr)
                    dst = pl.multiple_of(src % rs, pr)
                    p_copy(src, dst, pr, it).start()
            return f
        np_ = ni * ur
        pins = [mk((s * np_) // nslots, ((s + 1) * np_) // nslots) for s in range(nslots)]
        compute(it, pins)
        return jw

    def step_b(it, jw):
        c_waits(it)

        @pl.when(it == nit - (lead + ur - 1) // ur)
        def _():
            last_b().wait()
        jw = p_wait(it, jw)
        base = s0 + spi * (it - sa)

        def first():
            for k in range(spi):
                strip(base + k).start()
        compute(it, [first] + [None] * (nslots - 1))
        return jw

    with _scope("loopA"):
        jw = jax.lax.fori_loop(0, sa, step_a, jnp.int32(0))
    with _scope("waitR"):
        last_a().wait()
    with _scope("startW"):
        start_strips(0, s0)
    with _scope("loopB"):
        jax.lax.fori_loop(sa, nit, step_b, jw)
    with _scope("tail"):
        start_strips(n_in_loop, nstrips)
        pltpu.make_async_copy(cbuf, o_hbm, wsem).wait()


@jax.jit
def pallas_standalone__detection_seg_fpn_lateral__vision_kernel(
    c_fine: jax.Array,
    p_coarse: jax.Array,
    w_lat: jax.Array,
    w_out: jax.Array,
):
    cfg = CFG
    B, H, W, C = c_fine.shape
    npairs = B * H // 2
    c3 = c_fine.reshape(npairs, 2 * W, C)
    p2 = p_coarse.reshape(npairs * (W // 2), C)
    wo = w_out.reshape(C, C)
    any_spec = pl.BlockSpec(memory_space=pl.ANY)
    out = pl.pallas_call(
        functools.partial(_kernel, **cfg),
        in_specs=[any_spec] * 4,
        out_specs=any_spec,
        out_shape=jax.ShapeDtypeStruct((npairs, 2 * W, C), c_fine.dtype),
        scratch_shapes=[
            pltpu.VMEM((npairs, 2 * W, C), jnp.bfloat16),
            pltpu.VMEM((cfg["pring"] * (W // 2) + 16, C), jnp.bfloat16),
            pltpu.VMEM((C, C), jnp.bfloat16),
            pltpu.VMEM((C, C), jnp.bfloat16),
            pltpu.VMEM((C, C), jnp.bfloat16),
            pltpu.VMEM((cfg["ur"], C // 128, W, 128), jnp.float32),
            pltpu.SemaphoreType.DMA((npairs // cfg["u"] + 2,)),
            pltpu.SemaphoreType.DMA((cfg["sa"] + 1,)),
            pltpu.SemaphoreType.DMA(()),
            pltpu.SemaphoreType.DMA((2,)),
        ],
        compiler_params=pltpu.CompilerParams(vmem_limit_bytes=127 * 1024 * 1024,
                                             disable_bounds_checks=True),
    )(c3, p2, w_lat, wo)
    return out.reshape(B, H, W, C)
```

```python
import functools

import jax
import jax.numpy as jnp
import jax.experimental.pallas as pl
import jax.experimental.pallas.tpu as pltpu

CFG = dict(
    ur=2,
    cq=11,
    pring=90,
    pr=32,
    npc=20,
    cr=48,
    ncp=16,
    merge=True,
    sa=57,
    sw=4096,
    wg=6,
    bw=32,
    s0=16,
    spi=16,
    mc=96,
    qc=96,
    lead=640,
    dist=1,
)
SCOPES = False


class _NoScope:
    def __enter__(self):
        return self

    def __exit__(self, *a):
        return False


def _scope(name):
    return jax.named_scope(name) if SCOPES else _NoScope()


def _spread(n_a, n_b, nslots, merge):
    slots = [[] for _ in range(nslots)]
    if merge:
        for k in range(n_a):
            slots[(k * nslots) // n_a].append(("a", k))
        for k in range(n_b):
            slots[((2 * k + 1) * nslots) // (2 * n_b)].append(("b", k))
    else:
        items = sorted([((k + 0.25) / n_a, "a", k) for k in range(n_a)]
                       + [((k + 0.75) / max(n_b, 1), "b", k) for k in range(n_b)])
        for j, (_, t, k) in enumerate(items):
            slots[(j * nslots) // len(items)].append((t, k))
    return slots


def _kernel(c_hbm, p_hbm, wl_hbm, wo_hbm, o_hbm,
            cbuf, pbuf, wl_v, wo_v, wf_v, up_ref, csem, psem, isem, wsem, ksem,
            *, W, ur, cq, pring, pr, npc, cr, ncp, merge, sa, sw, wg, bw, s0, spi, mc, qc,
            lead, dist):
    nrows, C = c_hbm.shape
    w2 = 2 * W
    WP = W // 2
    npairs = nrows // w2
    nt = C // 128
    nit = npairs // ur
    ru = ur * w2
    ns = sw // bw
    nstrips = (nrows // (wg * sw)) * ns
    cview = cbuf.reshape(nrows // sw, sw, C)
    ptot = npairs * WP
    rs = pring * WP
    fpi = npc * pr
    f0 = ptot - fpi * sa
    cpi = ncp * cr
    rbulk = nrows - cpi * sa
    nfull = (rbulk - lead - 1) // ru
    exact = f0 % WP == 0 and rs % fpi == 0
    shift = rs - f0 if exact else 0
    assert f0 >= ur * WP and f0 % pr == 0 and rs % pr == 0 and f0 <= rs
    assert fpi >= ur * WP
    for it in range(sa):
        assert f0 + fpi * (it + 1) - rs <= ur * it * WP
    assert cq + sa - 1 >= nfull
    assert nfull >= sa
    n_in_loop = s0 + spi * (nit - sa)
    assert n_in_loop <= nstrips
    for it in range(sa, nit):
        hi = s0 + spi * (it - sa + 1)
        assert -(-hi // ns) * wg * sw <= it * ru, it
    anchor = rs

    def c_copy(lo, n, sem):
        return pltpu.make_async_copy(c_hbm.at[pl.ds(lo, n)], cbuf.at[pl.ds(lo, n)], sem)

    def rd_c(un):
        return c_copy(pl.multiple_of(un * ru, ru), ru, csem.at[un])

    def last_a():
        return c_copy(nfull * ru, rbulk - lead - nfull * ru, csem.at[nfull])

    def last_b():
        return c_copy(rbulk - lead, lead, csem.at[nfull + 1])

    def p_copy(src, n, sem):
        dst = pl.multiple_of((src + shift) % rs, 16)
        return pltpu.make_async_copy(p_hbm.at[pl.ds(src, n)], pbuf.at[pl.ds(dst, n)], sem)

    def strip(t):
        g = t // ns
        off = pl.multiple_of((t % ns) * bw, bw)
        return pltpu.make_async_copy(
            cview.at[pl.ds(g * wg, wg), pl.ds(off, bw)],
            o_hbm.at[pl.ds(g * wg, wg), pl.ds(off, bw)], wsem)

    def start_strips(lo, hi):
        def issue(t, carry):
            strip(t).start()
            return carry
        jax.lax.fori_loop(lo, hi, issue, 0)

    wl_cp = pltpu.make_async_copy(wl_hbm, wl_v, ksem.at[0])
    wo_cp = pltpu.make_async_copy(wo_hbm, wo_v, ksem.at[1])
    wl_cp.start()
    wo_cp.start()
    p_first = p_copy(0, f0, psem.at[sa])
    p_first.start()

    def pro_c(un, carry):
        rd_c(un).start(priority=1)
        return carry
    jax.lax.fori_loop(0, cq, pro_c, 0)

    with _scope("fold"):
        wl_cp.wait()
        wo_cp.wait()
        wf_v[...] = jnp.dot(
            wl_v[...], wo_v[...],
            preferred_element_type=jnp.float32).astype(jnp.bfloat16)
        p_first.wait()

    def p_wait(it, jw):
        need = f0 + fpi * jw < ur * WP * (it + 1)

        @pl.when(need)
        def _():
            if exact:
                p_copy(pl.multiple_of(f0 + fpi * jw, 16), fpi, psem.at[jw]).wait()
            else:
                pltpu.make_async_copy(p_hbm.at[pl.ds(0, fpi)], pbuf.at[pl.ds(0, fpi)],
                                      psem.at[jw]).wait()
        return jw + need.astype(jnp.int32)

    def compute(it, pins):
        pins = iter(pins)

        def pin(tile):
            f = next(pins)
            if f is not None:
                if tile is not None:
                    pbuf[pl.ds(anchor, 16), pl.ds(0, 128)] = tile
                f()

        prows = []
        for k in range(ur):
            prow = pl.multiple_of(((it * ur + k) * WP + shift) % rs, WP)
            prows.append(pbuf[pl.ds(prow, WP), :])
        nch = w2 // mc
        njobs = ur * nch
        base = pl.multiple_of(it * ru, ru)
        lhs = {}

        def load(j):
            if j < njobs:
                lhs[j] = cbuf[pl.ds(base + j * mc, mc), :]

        for j in range(dist):
            load(j)
        pin(None)
        for j in range(njobs):
            k, ch = divmod(j, nch)
            if ch == 0:
                for qh in range(WP // qc):
                    q = jnp.dot(prows[k][qh * qc:(qh + 1) * qc], wo_v[...],
                                preferred_element_type=jnp.float32)
                    for n in range(nt):
                        qn = q[:, n * 128:(n + 1) * 128]
                        up_ref[k, n, pl.ds(2 * qh * qc, qc, stride=2), :] = qn
                        up_ref[k, n, pl.ds(2 * qh * qc + 1, qc, stride=2), :] = qn
                    pin(q[0:16, 0:128].astype(jnp.bfloat16))
            load(j + dist)
            acc = jnp.dot(lhs.pop(j), wf_v[...], preferred_element_type=jnp.float32)
            uo = (ch * mc) % W
            up = jnp.concatenate([up_ref[k, n, pl.ds(uo, mc), :] for n in range(nt)], axis=1)
            res = (acc + up).astype(cbuf.dtype)
            cbuf[pl.ds(base + j * mc, mc), :] = res
            if j < njobs - 1:
                pin(res[0:16, 0:128])

    nslots = ur * (WP // qc + w2 // mc)
    plan = _spread(npc, ncp, nslots, merge)

    def step_a(it, jw):
        un = it + cq

        @pl.when(un < nfull)
        def _():
            rd_c(un).start(priority=1)

        @pl.when(un == nfull)
        def _():
            last_a().start(priority=1)
            last_b().start(priority=1)

        with _scope("waitC"):
            rd_c(it).wait()
        jw = p_wait(it, jw)

        def mk(items):
            if not items:
                return None

            def f():
                for t, k in items:
                    if t == "a":
                        src = pl.multiple_of(f0 + fpi * it + k * pr, 16)
                        p_copy(src, pr, psem.at[it]).start()
                    else:
                        src = pl.multiple_of(rbulk + cpi * it + k * cr, 16)
                        c_copy(src, cr, isem).start()
            return f
        compute(it, [mk(items) for items in plan])
        return jw

    def step_b(it, jw):
        @pl.when(it < nfull)
        def _():
            rd_c(it).wait()

        @pl.when(it == nfull)
        def _():
            last_b().wait()
            if cpi:
                c_copy(rbulk, cpi * sa, isem).wait()
        jw = p_wait(it, jw)
        base = s0 + spi * (it - sa)

        def first():
            for k in range(spi):
                strip(base + k).start()
        compute(it, [first] + [None] * (nslots - 1))
        return jw

    with _scope("loopA"):
        jw = jax.lax.fori_loop(0, sa, step_a, jnp.int32(0))
    with _scope("waitR"):
        last_a().wait()
    with _scope("startW"):
        start_strips(0, s0)
    with _scope("loopB"):
        jax.lax.fori_loop(sa, nit, step_b, jw)
    with _scope("tail"):
        start_strips(n_in_loop, nstrips)
        pltpu.make_async_copy(cview, o_hbm, wsem).wait()


@jax.jit
def pallas_standalone__detection_seg_fpn_lateral__vision_kernel(
    c_fine: jax.Array,
    p_coarse: jax.Array,
    w_lat: jax.Array,
    w_out: jax.Array,
):
    cfg = CFG
    B, H, W, C = c_fine.shape
    nrows = B * H * W
    c2 = c_fine.reshape(nrows, C)
    p2 = p_coarse.reshape(nrows // 4, C)
    wo = w_out.reshape(C, C)
    any_spec = pl.BlockSpec(memory_space=pl.ANY)
    out = pl.pallas_call(
        functools.partial(_kernel, W=W, **cfg),
        in_specs=[any_spec] * 4,
        out_specs=any_spec,
        out_shape=jax.ShapeDtypeStruct((nrows // cfg["sw"], cfg["sw"], C), c_fine.dtype),
        scratch_shapes=[
            pltpu.VMEM((nrows, C), jnp.bfloat16),
            pltpu.VMEM((cfg["pring"] * (W // 2) + 16, C), jnp.bfloat16),
            pltpu.VMEM((C, C), jnp.bfloat16),
            pltpu.VMEM((C, C), jnp.bfloat16),
            pltpu.VMEM((C, C), jnp.bfloat16),
            pltpu.VMEM((cfg["ur"], C // 128, W, 128), jnp.float32),
            pltpu.SemaphoreType.DMA((B * H // (2 * cfg["ur"]) + 2,)),
            pltpu.SemaphoreType.DMA((cfg["sa"] + 1,)),
            pltpu.SemaphoreType.DMA(()),
            pltpu.SemaphoreType.DMA(()),
            pltpu.SemaphoreType.DMA((2,)),
        ],
        compiler_params=pltpu.CompilerParams(vmem_limit_bytes=127 * 1024 * 1024,
                                             disable_bounds_checks=True,
                                             disable_semaphore_checks=True),
    )(c2, p2, w_lat, wo)
    return out.reshape(B, H, W, C)
```

```python
import functools

import jax
import jax.numpy as jnp
import jax.experimental.pallas as pl
import jax.experimental.pallas.tpu as pltpu

CFG = dict(
    ur=2,
    gp=8,
    rr=16,
    pblk=24,
    rpi=20,
    sa=53,
    lead=5,
    rf=44,
    sw=2048,
    wg=6,
    bw=16,
    s0=32,
    spi=32,
    wb=4,
    mc=96,
    qc=96,
)
SCOPES = False


class _NoScope:
    def __enter__(self):
        return self

    def __exit__(self, *a):
        return False


def _scope(name):
    return jax.named_scope(name) if SCOPES else _NoScope()


def _kernel(c_hbm, p_hbm, wl_hbm, wo_hbm, o_hbm,
            cbuf, pbuf, wl_v, wo_v, wf_v, up_ref, rsem, wsem, ksem,
            *, ur, gp, rr, pblk, rpi, sa, lead, rf, sw, wg, bw, s0, spi, wb, mc, qc):
    npairs, w2, C = c_hbm.shape
    W = w2 // 2
    WP = W // 2
    nrows = npairs * w2
    nt = C // 128
    nit = npairs // ur
    ru = ur * w2
    ppb = w2 // WP
    gb = gp // ppb
    ng = npairs // gp
    ipg = gp // ur
    rpg = w2 // rr
    nreps = ng * rpg
    r0 = nreps - rpi * sa
    ns = sw // bw
    nstrips = (nrows // (wg * sw)) * ns
    nch = w2 // mc
    njobs = ur * nch
    cv = cbuf.reshape(npairs, w2, C)
    ov = cbuf.reshape(nrows // sw, sw, C)

    assert gp % ppb == 0 and gp % ur == 0 and pblk % gb == 0 and rpg <= r0 and rf <= r0
    for it in range(sa):
        g_hi = (r0 + rpi * (it + 1) - 1) // rpg
        assert (g_hi + 1) * gp - pblk * ppb <= ur * it
        assert (it // ipg + 1) * rpg <= r0 + rpi * it
    assert sa <= (ng - 1) * ipg
    n_in_loop = s0 + spi * (nit - sa)
    assert n_in_loop <= nstrips
    for it in range(sa, nit):
        hi = s0 + spi * (it - sa + 1)
        assert -(-hi // ns) * wg * sw <= it * ru

    def c_copy(g, off, n, s):
        sl = (pl.ds(g * gp, gp), pl.ds(off, n))
        return pltpu.make_async_copy(c_hbm.at[sl], cv.at[sl], rsem.at[s])

    def p_copy(g, off, n):
        slot = (g * gb) % pblk
        return pltpu.make_async_copy(
            p_hbm.at[pl.ds(g * gb, gb), pl.ds(off, n)],
            pbuf.at[pl.ds(slot, gb), pl.ds(off, n)], rsem.at[ng + 1 + g])

    def start_rep(r):
        g = r // rpg
        off = pl.multiple_of((r % rpg) * rr, rr)
        s = g + (r >= nreps - lead).astype(jnp.int32)
        c_copy(g, off, rr, s).start(priority=1)
        p_copy(g, off, rr).start()

    def start_reps(lo, hi):
        def issue(r, carry):
            start_rep(r)
            return carry
        jax.lax.fori_loop(lo, hi, issue, 0)

    def start_strip(t):
        g = t // ns
        off = pl.multiple_of((t % ns) * bw, bw)
        sl = (pl.ds(g * wg, wg), pl.ds(off, bw))
        pltpu.make_async_copy(ov.at[sl], o_hbm.at[sl], wsem).start()

    def start_strips(lo, hi):
        def issue(t, carry):
            start_strip(t)
            return carry
        jax.lax.fori_loop(lo, hi, issue, 0)

    wl_cp = pltpu.make_async_copy(wl_hbm, wl_v, ksem.at[0])
    wo_cp = pltpu.make_async_copy(wo_hbm, wo_v, ksem.at[1])
    wl_cp.start()
    wo_cp.start()
    start_reps(0, rf)
    with _scope("fold"):
        wl_cp.wait()
        wo_cp.wait()
        wf_v[...] = jnp.dot(
            wl_v[...], wo_v[...],
            preferred_element_type=jnp.float32).astype(jnp.bfloat16)
    with _scope("pro"):
        start_reps(rf, r0)

    def group_waits(it):
        g = it // ipg

        @pl.when(it % ipg == 0)
        def _():
            with _scope("waitG"):
                p_copy(g, 0, w2).wait()

                @pl.when(g < ng - 1)
                def _():
                    c_copy(g, 0, w2, g).wait()

                @pl.when(g == ng - 1)
                def _():
                    c_copy(ng - 1, w2 - lead * rr, lead * rr, ng).wait()

    def compute(it, before, after):
        base = pl.multiple_of(it * ru, ru)

        def p_row(k):
            i = it * ur + k
            off = pl.multiple_of((i % ppb) * WP, WP)
            return pbuf[(i // ppb) % pblk, pl.ds(off, WP), :]

        def c_chunk(j):
            return cbuf[pl.ds(base + j * mc, mc), :]

        prow = p_row(0)
        lhs = c_chunk(0)
        for j in range(njobs):
            k, ch = divmod(j, nch)
            before(j)
            if ch == 0:
                for h in range(WP // qc):
                    q = jnp.dot(prow[h * qc:(h + 1) * qc], wo_v[...],
                                preferred_element_type=jnp.float32)
                    for n in range(nt):
                        qn = q[:, n * 128:(n + 1) * 128]
                        up_ref[k, n, pl.ds(2 * h * qc, qc, stride=2), :] = qn
                        up_ref[k, n, pl.ds(2 * h * qc + 1, qc, stride=2), :] = qn
            cur = lhs
            if j + 1 < njobs:
                lhs = c_chunk(j + 1)
            if ch == nch - 1 and k + 1 < ur:
                prow = p_row(k + 1)
            acc = jnp.dot(cur, wf_v[...], preferred_element_type=jnp.float32)
            uo = (ch * mc) % W
            up = jnp.concatenate(
                [up_ref[k, n, pl.ds(uo, mc), :] for n in range(nt)], axis=1)
            cbuf[pl.ds(base + j * mc, mc), :] = (acc + up).astype(cbuf.dtype)
            after(j)

    def nothing(j):
        pass

    def read_step(it, carry):
        group_waits(it)

        def after(j):
            for k in range(-(-j * rpi // njobs), -(-(j + 1) * rpi // njobs)):
                start_rep(r0 + rpi * it + k)
        compute(it, nothing, after)
        return carry

    def write_step(it, carry):
        group_waits(it)

        def before(j):
            if j % (njobs // wb) == 0:
                b = j // (njobs // wb)
                for k in range((b * spi) // wb, ((b + 1) * spi) // wb):
                    start_strip(s0 + spi * (it - sa) + k)
        compute(it, before, nothing)
        return carry

    with _scope("loopA"):
        jax.lax.fori_loop(0, sa, read_step, 0)
    with _scope("waitR"):
        c_copy(ng - 1, 0, w2 - lead * rr, ng - 1).wait()
    with _scope("startW"):
        start_strips(0, s0)
    with _scope("loopB"):
        jax.lax.fori_loop(sa, nit, write_step, 0)
    with _scope("tail"):
        start_strips(n_in_loop, nstrips)
        pltpu.make_async_copy(ov, o_hbm, wsem).wait()


@jax.jit
def pallas_standalone__detection_seg_fpn_lateral__vision_kernel(
    c_fine: jax.Array,
    p_coarse: jax.Array,
    w_lat: jax.Array,
    w_out: jax.Array,
):
    cfg = CFG
    B, H, W, C = c_fine.shape
    nrows = B * H * W
    npairs = B * H // 2
    c3 = c_fine.reshape(npairs, 2 * W, C)
    p3 = p_coarse.reshape(npairs // 4, 2 * W, C)
    wo = w_out.reshape(C, C)
    any_spec = pl.BlockSpec(memory_space=pl.ANY)
    out = pl.pallas_call(
        functools.partial(_kernel, **cfg),
        in_specs=[any_spec] * 4,
        out_specs=any_spec,
        out_shape=jax.ShapeDtypeStruct((nrows // cfg["sw"], cfg["sw"], C), c_fine.dtype),
        scratch_shapes=[
            pltpu.VMEM((nrows, C), jnp.bfloat16),
            pltpu.VMEM((cfg["pblk"], 2 * W, C), jnp.bfloat16),
            pltpu.VMEM((C, C), jnp.bfloat16),
            pltpu.VMEM((C, C), jnp.bfloat16),
            pltpu.VMEM((C, C), jnp.bfloat16),
            pltpu.VMEM((cfg["ur"], C // 128, W, 128), jnp.float32),
            pltpu.SemaphoreType.DMA((2 * (npairs // cfg["gp"]) + 1,)),
            pltpu.SemaphoreType.DMA(()),
            pltpu.SemaphoreType.DMA((2,)),
        ],
        compiler_params=pltpu.CompilerParams(vmem_limit_bytes=127 * 1024 * 1024,
                                             disable_bounds_checks=True,
                                             disable_semaphore_checks=True),
    )(c3, p3, w_lat, wo)
    return out.reshape(B, H, W, C)
```

```python
import functools

import jax
import jax.numpy as jnp
import jax.experimental.pallas as pl
import jax.experimental.pallas.tpu as pltpu

CFG = dict(
    ur=2,
    gp=8,
    rr=16,
    pblk=24,
    rpi=20,
    sa=53,
    lead=5,
    rf=44,
    sw=2048,
    wg=6,
    bw=16,
    s0=32,
    spi=32,
    wb=4,
    mc=96,
    qc=96,
)


def _kernel(c_hbm, p_hbm, wl_hbm, wo_hbm, o_hbm,
            cbuf, pbuf, wl_v, wo_v, wf_v, up_ref, rsem, wsem, ksem,
            *, ur, gp, rr, pblk, rpi, sa, lead, rf, sw, wg, bw, s0, spi, wb, mc, qc):
    npairs, w2, C = c_hbm.shape
    W = w2 // 2
    WP = W // 2
    nrows = npairs * w2
    nt = C // 128
    nit = npairs // ur
    ru = ur * w2
    ppb = w2 // WP
    gb = gp // ppb
    ng = npairs // gp
    ipg = gp // ur
    rpg = w2 // rr
    nreps = ng * rpg
    r0 = nreps - rpi * sa
    ns = sw // bw
    nstrips = (nrows // (wg * sw)) * ns
    nch = w2 // mc
    njobs = ur * nch
    ov = cbuf if sw == w2 else cbuf.reshape(nrows // sw, sw, C)

    assert gp % ppb == 0 and gp % ur == 0 and pblk % gb == 0 and rpg <= r0 and rf <= r0
    for it in range(sa):
        g_hi = (r0 + rpi * (it + 1) - 1) // rpg
        assert (g_hi + 1) * gp - pblk * ppb <= ur * it
        assert (it // ipg + 1) * rpg <= r0 + rpi * it
    assert sa <= (ng - 1) * ipg
    n_in_loop = s0 + spi * (nit - sa)
    assert n_in_loop <= nstrips
    for it in range(sa, nit):
        hi = s0 + spi * (it - sa + 1)
        assert -(-hi // ns) * wg * sw <= it * ru

    def c_copy(g, off, n, s):
        sl = (pl.ds(g * gp, gp), pl.ds(off, n))
        return pltpu.make_async_copy(c_hbm.at[sl], cbuf.at[sl], rsem.at[s])

    def p_copy(g, off, n):
        slot = (g * gb) % pblk
        return pltpu.make_async_copy(
            p_hbm.at[pl.ds(g * gb, gb), pl.ds(off, n)],
            pbuf.at[pl.ds(slot, gb), pl.ds(off, n)], rsem.at[ng + 1 + g])

    def start_rep(r):
        g = r // rpg
        off = pl.multiple_of((r % rpg) * rr, rr)
        s = g + (r >= nreps - lead).astype(jnp.int32)
        c_copy(g, off, rr, s).start(priority=1)
        p_copy(g, off, rr).start()

    def start_reps(lo, hi):
        def issue(r, carry):
            start_rep(r)
            return carry
        jax.lax.fori_loop(lo, hi, issue, 0)

    def start_strip(t):
        g = t // ns
        off = pl.multiple_of((t % ns) * bw, bw)
        sl = (pl.ds(g * wg, wg), pl.ds(off, bw))
        pltpu.make_async_copy(ov.at[sl], o_hbm.at[sl], wsem).start()

    def start_strips(lo, hi):
        def issue(t, carry):
            start_strip(t)
            return carry
        jax.lax.fori_loop(lo, hi, issue, 0)

    wl_cp = pltpu.make_async_copy(wl_hbm, wl_v, ksem.at[0])
    wo_cp = pltpu.make_async_copy(wo_hbm, wo_v, ksem.at[1])
    wl_cp.start()
    wo_cp.start()
    start_reps(0, rf)
    wl_cp.wait()
    wo_cp.wait()
    wf_v[...] = jnp.dot(
        wl_v[...], wo_v[...],
        preferred_element_type=jnp.float32).astype(jnp.bfloat16)
    start_reps(rf, r0)

    def group_waits(it):
        g = it // ipg

        @pl.when(it % ipg == 0)
        def _():
            p_copy(g, 0, w2).wait()

            @pl.when(g < ng - 1)
            def _():
                c_copy(g, 0, w2, g).wait()

            @pl.when(g == ng - 1)
            def _():
                c_copy(ng - 1, w2 - lead * rr, lead * rr, ng).wait()

    def compute(it, before, after):
        def p_row(k):
            i = it * ur + k
            off = pl.multiple_of((i % ppb) * WP, WP)
            return pbuf[(i // ppb) % pblk, pl.ds(off, WP), :]

        def c_chunk(j):
            return cbuf[it * ur + j // nch, pl.ds((j % nch) * mc, mc), :]

        prow = p_row(0)
        lhs = c_chunk(0)
        for j in range(njobs):
            k, ch = divmod(j, nch)
            before(j)
            if ch == 0:
                for h in range(WP // qc):
                    q = jnp.dot(prow[h * qc:(h + 1) * qc], wo_v[...],
                                preferred_element_type=jnp.float32)
                    for n in range(nt):
                        qn = q[:, n * 128:(n + 1) * 128]
                        up_ref[k, n, pl.ds(2 * h * qc, qc, stride=2), :] = qn
                        up_ref[k, n, pl.ds(2 * h * qc + 1, qc, stride=2), :] = qn
            cur = lhs
            if j + 1 < njobs:
                lhs = c_chunk(j + 1)
            if ch == nch - 1 and k + 1 < ur:
                prow = p_row(k + 1)
            acc = jnp.dot(cur, wf_v[...], preferred_element_type=jnp.float32)
            uo = (ch * mc) % W
            up = jnp.concatenate(
                [up_ref[k, n, pl.ds(uo, mc), :] for n in range(nt)], axis=1)
            cbuf[it * ur + k, pl.ds(ch * mc, mc), :] = (acc + up).astype(cbuf.dtype)
            after(j)

    def nothing(j):
        pass

    def read_step(it, carry):
        group_waits(it)

        def after(j):
            for k in range(-(-j * rpi // njobs), -(-(j + 1) * rpi // njobs)):
                start_rep(r0 + rpi * it + k)
        compute(it, nothing, after)
        return carry

    def write_step(it, carry):
        group_waits(it)

        def before(j):
            if j % (njobs // wb) == 0:
                b = j // (njobs // wb)
                for k in range((b * spi) // wb, ((b + 1) * spi) // wb):
                    start_strip(s0 + spi * (it - sa) + k)
        compute(it, before, nothing)
        return carry

    jax.lax.fori_loop(0, sa, read_step, 0)
    c_copy(ng - 1, 0, w2 - lead * rr, ng - 1).wait()
    start_strips(0, s0)
    jax.lax.fori_loop(sa, nit, write_step, 0)
    start_strips(n_in_loop, nstrips)
    pltpu.make_async_copy(ov, o_hbm, wsem).wait()


@jax.jit
def pallas_standalone__detection_seg_fpn_lateral__vision_kernel(
    c_fine: jax.Array,
    p_coarse: jax.Array,
    w_lat: jax.Array,
    w_out: jax.Array,
):
    cfg = CFG
    B, H, W, C = c_fine.shape
    nrows = B * H * W
    npairs = B * H // 2
    c3 = c_fine.reshape(npairs, 2 * W, C)
    p3 = p_coarse.reshape(npairs // 4, 2 * W, C)
    wo = w_out.reshape(C, C)
    any_spec = pl.BlockSpec(memory_space=pl.ANY)
    out = pl.pallas_call(
        functools.partial(_kernel, **cfg),
        in_specs=[any_spec] * 4,
        out_specs=any_spec,
        out_shape=jax.ShapeDtypeStruct((nrows // cfg["sw"], cfg["sw"], C), c_fine.dtype),
        scratch_shapes=[
            pltpu.VMEM((npairs, 2 * W, C), jnp.bfloat16),
            pltpu.VMEM((cfg["pblk"], 2 * W, C), jnp.bfloat16),
            pltpu.VMEM((C, C), jnp.bfloat16),
            pltpu.VMEM((C, C), jnp.bfloat16),
            pltpu.VMEM((C, C), jnp.bfloat16),
            pltpu.VMEM((cfg["ur"], C // 128, W + 8, 128), jnp.float32),
            pltpu.SemaphoreType.DMA((2 * (npairs // cfg["gp"]) + 1,)),
            pltpu.SemaphoreType.DMA(()),
            pltpu.SemaphoreType.DMA((2,)),
        ],
        compiler_params=pltpu.CompilerParams(vmem_limit_bytes=127 * 1024 * 1024,
                                             disable_bounds_checks=True,
                                             disable_semaphore_checks=True),
    )(c3, p3, w_lat, wo)
    return out.reshape(B, H, W, C)
```
